```python
import os as _os
_os.environ.setdefault("JAX_PLATFORMS", "cpu")
import jax
import jax.numpy as jnp

def _softmax(x, axis=-1):
    return jax.nn.softmax(x, axis=axis)
def _gelu(x):
    return jax.nn.gelu(x, approximate=True)
def _silu(x):
    return jax.nn.silu(x)
def _sigmoid(x):
    return jax.nn.sigmoid(x)
def _layernorm(x, axis=-1, eps=1e-5):
    m = jnp.mean(x, axis=axis, keepdims=True)
    v = jnp.var(x, axis=axis, keepdims=True)
    return (x - m) / jnp.sqrt(v + eps)
def _scatter_add(tgt, idx, src, axis=0):
    return tgt.at[idx].add(src)
def _segment_sum(src, seg, n):
    return jax.ops.segment_sum(src, seg, n)
class _Rng:
    def __init__(self, key):
        self._k = key
    def _next(self):
        self._k, sub = jax.random.split(self._k)
        return sub
    def normal(self, shape):
        return jax.random.normal(self._next(), shape, dtype=jnp.bfloat16)
    def randint(self, lo, hi, shape):
        return jax.random.randint(self._next(), shape, lo, hi, dtype=jnp.int32)
    def uniform(self, shape, lo=0.0, hi=1.0):
        return jax.random.uniform(self._next(), shape, jnp.bfloat16, lo, hi)
    def permutation(self, n):
        return jax.random.permutation(self._next(), n)


kernel_name = 'standalone__layernorm_linear__sampling'

def setup_inputs():
    _rng = _Rng(jax.random.key(int.from_bytes(__import__("os").urandom(4), "little")))
    _w = (lambda a: (lambda t: t.astype(jnp.bfloat16) if jnp.issubdtype(t.dtype, jnp.floating) else t)(jnp.asarray(a)))
    B, S, D = 1024, 32, 576
    return {
        "x": _w((lambda *s: _rng.normal(s) * 0.05)(B, S, D)),
        "g": _w((lambda *s: _rng.normal(s) * 0.05)(D) + 1.0),
        "b": _w((lambda *s: _rng.normal(s) * 0.05)(D)),
        "w": _w((lambda *s: _rng.normal(s) * 0.05)(D, D)),
    }

def reference(x, g, b, w):
    return (_layernorm(x, axis=-1) * g + b) @ w
```

```python
import functools
import itertools

import jax
import jax.numpy as jnp
from jax import lax
import jax.experimental.pallas as pl
import jax.experimental.pallas.tpu as pltpu

F32, BF16, U32 = jnp.float32, jnp.bfloat16, jnp.uint32
EPS = 1e-5
NH = 256
NG = 2 * NH

TILES = ["1a", "1b", "6a", "6b", "7a", "7b", "5a", "5b", "2a", "2b", "2c", "3a", "3b", "3c", "4a", "4b", "4c"]
RHS = {
    "1a": [("X1", 0, 128)], "1b": [("X1", 256, 64), ("ONE", 0, 64)],
    "6a": [("T2", 0, 128)], "6b": [("T2", 256, 64), ("X2", 512, 64)],
    "7a": [("T3", 0, 128)], "7b": [("T3", 256, 64), ("X2", 448, 64)],
    "5a": [("D21", 0, 128)], "5b": [("D21", 256, 64), ("X2", 320, 64)],
    "2a": [("X1", 128, 128)], "2b": [("X1", 384, 128)], "2c": [("X1", 512, 64), ("X1", 320, 64)],
    "3a": [("X2", 128, 128)], "3b": [("X2", 384, 128)], "3c": [("X2", 512, 64), ("X2", 320, 64)],
    "4a": [("T4", 0, 128)], "4b": [("T4", 256, 64), ("D12", 448, 64)], "4c": [("D12", 512, 64), ("X1", 320, 64)],
}
cat0 = lambda xs: jnp.concatenate(xs, axis=0) if len(xs) > 1 else xs[0]
cat1 = lambda xs: jnp.concatenate(xs, axis=1) if len(xs) > 1 else xs[0]
add_all = lambda xs: functools.reduce(lambda a, b: a + b, xs)


def make(blocks=((1, 2), (2, 1), (4, 7)), wstart=13, r1=32, r2=16, jr=32, rw=(0, 1, 2, 1, 2, 1, 1, 2, 0), stage=False, dma=True, flags=None):
    def fn(x, g, b, w):
        B, S, D = x.shape
        H = D // 2
        G = B // NG
        NV = NG // 128

        def kern(x_hbm, g_hbm, b_hbm, w_hbm, o_hbm, xbuf, obuf, wbuf, gbuf, bbuf, lhs, bias, stat, part, xc, isem, osem, psem):
            def x_copy(k):
                sl = (k // G, slice(None), pl.ds((k % G) * NG, NG)) if k < G else (k - G + 1,)
                return pltpu.make_async_copy(x_hbm.at[sl], xbuf.at[sl], isem.at[k])
            params = [pltpu.make_async_copy(s, d, psem.at[i]) for i, (s, d) in enumerate(((g_hbm, gbuf), (b_hbm, bbuf), (w_hbm, wbuf)))]
            slab_copy = lambda s: pltpu.make_async_copy(x_hbm.at[s], xbuf.at[s], isem.at[s + G - 1])
            for c in params:
                c.start()

            @pl.loop(0, G)
            def _(k):
                sl = (0, slice(None), pl.ds(pl.multiple_of(k * NG, NG), NG))
                pltpu.make_async_copy(x_hbm.at[sl], xbuf.at[sl], isem.at[k]).start()

            if dma:
                @pl.loop(1, S)
                def _(s):
                    slab_copy(s).start()

            for c in params:
                c.wait()

            gr = gbuf[...].astype(F32).reshape(1, D)
            br = bbuf[...].astype(F32).reshape(1, D)
            lo = lax.broadcasted_iota(jnp.int32, (H, 128), 1) < 64
            lane = lax.broadcasted_iota(jnp.int32, (H, 128), 1)
            A1, A2, c = [], [], None
            for t in range(5):
                if t < 4:
                    wt, gt, bt = wbuf[t * 128:(t + 1) * 128, :], gr[:, t * 128:(t + 1) * 128], br[:, t * 128:(t + 1) * 128]
                else:
                    wt = cat0([wbuf[512:, :]] * 2)
                    gt = cat1([gr[:, 512:]] * 2)
                    bt = cat1([br[:, 512:], jnp.zeros((1, 64), F32)])
                a = wt.astype(F32).T
                c = a * bt if c is None else c + a * bt
                a = a * gt
                A1.append(a[:H]); A2.append(a[H:])
            c = jnp.sum(c, axis=1, keepdims=True)
            bias[...] = jnp.broadcast_to(c[H:] - c[:H], (H, 128))
            c1 = jnp.broadcast_to(c[:H], (H, 128))
            ch = c1.astype(BF16).astype(F32)
            cm = (c1 - ch).astype(BF16).astype(F32)
            cb = jnp.where(lane == 64, ch, jnp.where(lane == 65, cm, jnp.where(lane == 66, c1 - ch - cm, 0.0)))
            sel = lambda u, v: jnp.where(lo, u, v)
            S1a, S1b = A2[0] + A2[1], A2[2] + A2[3]
            S2a, S2b = S1a - A1[0], S1b - A1[2]
            L = {"1a": A1[0], "1b": sel(A1[2], cb), "6a": S2a, "6b": sel(S2b, A2[4]),
                 "7a": A1[0] - A2[0], "7b": sel(A1[2] - A2[2], A2[3]), "5a": S1a, "5b": sel(S1b, A2[2]),
                 "2a": A1[1], "2b": A1[3], "2c": sel(A1[4], A1[2]),
                 "3a": A1[1] - S2a, "3b": sel(A1[3] - S2b, A1[3]), "3c": sel(A1[4] - A2[4], A1[2] - A2[2]),
                 "4a": A2[1], "4b": A2[3], "4c": sel(A2[4], A2[2])}
            for i, t in enumerate(TILES):
                lhs[i] = pltpu.bitcast(L[t].astype(BF16), U32)

            ACC_HI = 6 * NV

            def stats_work(s, gi, par, acc_base):
                def aget(i): return cat1([stat[acc_base + (i * NV + j)] for j in range(NV)])
                def aput(i, v):
                    for j in range(NV): stat[acc_base + (i * NV + j)] = v[:, j * 128:(j + 1) * 128]
                def sput(k, v):
                    for j in range(NV): stat[(2 + 2 * par + k) * NV + j] = v[:, j * 128:(j + 1) * 128]
                ld = lambda r0, n: xbuf[s, pl.ds(r0, n), pl.ds(gi * NG, NG)].astype(F32)
                def p1(r0):
                    v = ld(r0, r1)
                    v = add_all([v[i:i + 8] for i in range(0, r1, 8)])
                    acc = v if r0 == 0 else aget(0) + v
                    if r0 + r1 == D:
                        acc = jnp.broadcast_to(jnp.sum(acc, axis=0, keepdims=True) * (1.0 / D), (8, NG))
                        if not stage: sput(0, acc)
                    aput(0, acc)
                def p2(r0):
                    m = aget(0)
                    v = ld(r0, r2)
                    d = [v[i:i + 8] - m for i in range(0, r2, 8)]
                    if stage: xc[par, r0:r0 + r2, :] = cat0(d)
                    sq = add_all([u * u for u in d])
                    acc = sq if r0 == 0 else aget(1) + sq
                    if r0 + r2 == D:
                        var = jnp.sum(acc, axis=0, keepdims=True) * (1.0 / D)
                        acc = jnp.broadcast_to(lax.rsqrt(var + EPS), (8, NG))
                        sput(1, acc)
                    aput(1, acc)
                P = functools.partial
                return [(2 * r1, P(p1, r0)) for r0 in range(0, D, r1)] + [(4 * r2, P(p2, r0)) for r0 in range(0, D, r2)]

            def rhs_tiles(s, gi, par, names, hook):
                def piece(kind, r0, n):
                    if kind == "ONE": return jnp.ones((n, NH), F32)
                    sv = lambda k, h: cat0([cat1([stat[(2 + 2 * par + k) * NV + h * (NV // 2) + j] for j in range(NV // 2)])] * (n // 8))
                    if stage:
                        xr = lambda h, o: xc[par, r0 + o:r0 + o + n, h * NH:(h + 1) * NH]
                        xn = lambda h: xr(h, 0) * sv(1, h)
                    else:
                        xr = lambda h, o: xbuf[s, pl.ds(r0 + o, n), pl.ds(gi * NG + h * NH, NH)].astype(F32)
                        xn = lambda h: (xr(h, 0) - sv(0, h)) * sv(1, h)
                    df = lambda h: (xr(h, 128) - xr(h, 0)) * sv(1, h)
                    return dict(X1=lambda: xn(0), X2=lambda: xn(1), D21=lambda: xn(1) - xn(0), D12=lambda: xn(0) - xn(1),
                                T3=lambda: df(1), T2=lambda: df(1) + xn(0), T4=lambda: df(0) - df(1))[kind]()
                pcs = [[(k, r0 + o, jr) for k, r0, n in RHS[t] for o in range(0, n, jr)] for t in names]
                v = [[None] * len(p) for p in pcs]
                for i in reversed(range(128 // jr)):
                    for j in range(len(names)):
                        hook()
                        v[j][i] = piece(*pcs[j][i])
                return [cat0(u).astype(BF16) for u in v]

            def group(s, gi, par, bank, side, fine):
                def out(r0, h, v):
                    sl = (s, pl.ds(r0, v.shape[0]), pl.ds(gi * NG + h * NH, NH))
                    obuf[sl] = v.astype(BF16)
                    if fine and dma:
                        @pl.when(s >= wstart)
                        def _(): pltpu.make_async_copy(obuf.at[sl], o_hbm.at[sl], osem.at[0]).start()
                P1, U2, U3, U4 = (part.at[bank, k] for k in range(4))
                def f1(a, b): P1[...] = a + b
                def f6(a, b): U2[...] = P1[...] + (a + b)
                def f7(a, b): U3[...] = U2[...] + (a + b) + cat1([bias[...]] * (NH // 128))
                def f5(a, b):
                    m5 = a + b
                    out(H, 1, U3[...] + m5)
                    U4[...] = U2[...] + m5
                def f2(a, b): P1[...] = P1[...] + (a + b)
                def f4(a, b): U3[...] = U3[...] + (a + b)
                def f43(a, b):
                    out(H, 0, U3[...] + a)
                    U4[...] = U4[...] + b
                def f3(a, b): out(0, 1, U4[...] + (a + b))
                rounds = [(("1a", "1b"), f1), (("6a", "6b"), f6), (("7a", "7b"), f7), (("5a", "5b"), f5), (("2a", "2b"), f2),
                          (("4b", "4c"), f4), (("4a", "3a"), f43), (("3b", "3c"), f3), (("2c",), None)]
                total = sum(wt for wt, _ in side)
                cum = list(itertools.accumulate(rw[k] for k, (names, _) in enumerate(rounds) for _ in range(len(names) * 128 // jr)))
                st = dict(slot=0, pos=0, done=0)
                def hook():
                    want = cum[st["slot"]] * total / cum[-1] - 1e-6
                    st["slot"] += 1
                    while st["done"] < want:
                        wt, f = side[st["pos"]]
                        st["pos"] += 1; st["done"] += wt
                        f()
                mm = lambda t, r0, n, v: jnp.dot(pltpu.bitcast(lhs[TILES.index(t), r0 // 2:(r0 + n) // 2], BF16), v, preferred_element_type=F32)
                for names, post in rounds:
                    v = rhs_tiles(s, gi, par, names, hook)
                    if post is not None:
                        post(*(mm(t, 0, H, u) for t, u in zip(names, v)))
                    else:
                        lo_, hi_ = (mm(names[0], r0, H // 2, v[0]) for r0 in (0, H // 2))
                        out(0, 0, P1[...] + cat0([lo_, hi_]))
                assert st["pos"] == len(side)

            def block(it, s0, nslab, first):
                acc_base = jnp.minimum(it * ACC_HI, ACC_HI)
                bank = it & 1
                for q in range(nslab * G):
                    ds, gi = divmod(q, G)
                    dn, gn = divmod(q + 1, G)
                    if dn < nslab: side = stats_work(s0 + dn, gn, (q + 1) % 2, acc_base)
                    else: side = stats_work(jnp.where(it == 0, 0, jnp.minimum(s0 + dn, S - 1)), gn, (q + 1) % 2, acc_base)
                    lastslab = ds == nslab - 1
                    group(s0 + ds, gi, q % 2, bank, side, lastslab and gi == G - 1)
                    if dma:
                        s = s0 + ds
                        if gi == 0 and ds == (wstart - first) % nslab:
                            @pl.when(s == wstart)
                            def _(): pltpu.make_async_copy(obuf.at[pl.ds(0, wstart)], o_hbm.at[pl.ds(0, wstart)], osem.at[0]).start()
                        if lastslab and gi < G - 1:
                            sl = (s, slice(None), pl.ds(gi * NG, NG))
                        elif not lastslab and gi == G - 1:
                            sl = (s,)
                        else:
                            continue
                        @pl.when(s >= wstart)
                        def _(): pltpu.make_async_copy(obuf.at[sl], o_hbm.at[sl], osem.at[0]).start()

            x_copy(0).wait()
            for _, f in stats_work(0, 0, 0, 0): f()
            for k in range(1, G): x_copy(k).wait()

            @pl.loop(0, sum(reps for _, reps in blocks))
            def _(it):
                @pl.when(it == 1)
                def _():
                    if dma: slab_copy(blocks[0][0]).wait()
                    for _, f in stats_work(blocks[0][0], 0, 0, 0): f()
                first, it0 = 0, 0
                for nslab, reps in blocks:
                    @pl.when((it >= it0) & (it < it0 + reps))
                    def _():
                        s0 = first + (it - it0) * nslab
                        if dma:
                            for u in range(1, nslab): slab_copy(s0 + u).wait()
                            @pl.when((it > 0) & (s0 + nslab < S))
                            def _(): slab_copy(s0 + nslab).wait()
                        block(it, s0, nslab, first)
                    first += nslab * reps
                    it0 += reps
                assert first == S

            if dma:
                pltpu.make_async_copy(obuf, o_hbm, osem.at[0]).wait()
            else:
                c = pltpu.make_async_copy(obuf.at[0, pl.ds(0, 16)], o_hbm.at[0, pl.ds(0, 16)], osem.at[0]); c.start(); c.wait()

        hbm = pl.BlockSpec(memory_space=pl.ANY)
        out = pl.pallas_call(
            kern,
            in_specs=[hbm] * 4,
            out_specs=hbm,
            out_shape=jax.ShapeDtypeStruct((S, D, B), x.dtype),
            scratch_shapes=[pltpu.VMEM((S, D, B), BF16), pltpu.VMEM((S, D, B), BF16), pltpu.VMEM((D, D), BF16),
                            pltpu.VMEM((D,), BF16), pltpu.VMEM((D,), BF16),
                            pltpu.VMEM((17, H // 2, 128), U32), pltpu.VMEM((H, 128), F32), pltpu.VMEM((8 * NV, 8, 128), F32),
                            pltpu.VMEM((2, 4, H, NH), F32), pltpu.VMEM((2, D, NG), F32),
                            pltpu.SemaphoreType.DMA((S + G - 1,)), pltpu.SemaphoreType.DMA((1,)), pltpu.SemaphoreType.DMA((3,))],
            compiler_params=pltpu.CompilerParams(vmem_limit_bytes=110 << 20, flags=flags),
        )(jnp.transpose(x, (1, 2, 0)), g, b, w)
        return jnp.transpose(out, (2, 0, 1))
    return fn


_impl = make()


@jax.jit
def pallas_standalone__layernorm_linear__sampling_kernel(x, g, b, w):
    return _impl(x, g, b, w)
```

```python
import functools
import itertools

import jax
import jax.numpy as jnp
from jax import lax
import jax.experimental.pallas as pl
import jax.experimental.pallas.tpu as pltpu

F32, BF16, U32 = jnp.float32, jnp.bfloat16, jnp.uint32
EPS = 1e-5
NG = 512
cat0 = lambda xs: jnp.concatenate(xs, axis=0) if len(xs) > 1 else xs[0]
cat1 = lambda xs: jnp.concatenate(xs, axis=1) if len(xs) > 1 else xs[0]
add_all = lambda xs: functools.reduce(lambda a, b: a + b, xs)

def _form(kind, r):
    return {"X1": {(0, r): 1}, "X2": {(1, r): 1}, "D21": {(1, r): 1, (0, r): -1}, "D12": {(0, r): 1, (1, r): -1},
            "T3": {(1, r + 128): 1, (1, r): -1}, "T2": {(1, r + 128): 1, (1, r): -1, (0, r): 1},
            "T4": {(0, r + 128): 1, (0, r): -1, (1, r + 128): -1, (1, r): 1}, "Z": {}}[kind]
L1 = {
    "1a": [("X1", 0), ("X1", 64)], "1b": [("Z", 0), ("X1", 320)],
    "6a": [("T2", 0), ("T2", 64)], "6b": [("X2", 512), ("T2", 320)],
    "7a": [("T3", 0), ("T3", 64)], "7b": [("X2", 384), ("T3", 320)],
    "5a": [("D21", 0), ("D21", 64)], "5b": [("X2", 256), ("D21", 320)],
    "2a": [("X1", 128), ("X1", 192)], "2b": [("X1", 384), ("X1", 448)], "2c": [("X1", 256), ("X1", 512)],
    "3c": [("X2", 128), ("X2", 192)], "3b": [("X2", 384), ("X2", 448)], "3a": [("X2", 256), ("X2", 512)],
    "4c": [("T4", 0), ("T4", 64)], "4b": [("D12", 384), ("T4", 320)], "4a": [("X1", 256), ("D12", 512)],
}
def _rhs(t, j):
    return [{(2 * h + j, r): s for (h, r), s in _form(*p).items()} for p in L1[t]]
L2 = {1: ((("a", 0, 1), ("b", 1, 1)), (("a", 0, 1), ("b", 1, 1))),
      2: ((("a", 1, 1), ("b", 1, 1)), (("a", 0, 1),)),
      3: ((("a", 0, 1),), (("a", 1, 1), ("b", 1, -1))),
      4: ((("b", 1, 1),), (("b", 0, 1), ("a", 0, -1))),
      5: ((("a", 0, 1), ("b", 0, 1)), (("b", 1, 1),)),
      6: ((("a", 1, 1), ("a", 0, -1)), (("a", 0, 1), ("a", 1, 1))),
      7: ((("b", 0, 1), ("b", 1, -1)), (("b", 0, 1), ("b", 1, 1)))}
SWAP = {"1": 1, "2": 0, "3": 0, "4": 0}
def _rhs2(p, i):
    out = []
    for k in range(2):
        f = {}
        if any(_form(*L1[p + t][k]) for t, _, _ in L2[i][0]):
            for t, j, sg in L2[i][1]:
                f.update({key: s * sg for key, s in _rhs(p + t, j ^ SWAP[p])[k].items()})
        out.append(f)
    return out
FULL = ["2c", "3c", "4c", "5a", "5b", "6a", "6b", "7a", "7b"]


def make(blocks=((1, 2), (2, 1), (4, 7)), wk=30, lead=3, dr=24, r1=32, r2=16, jr=16, rw=(0, 9, 10, 0, 12, 10, 10, 2, 0, 1, 0, 0),
         dma=True, flags=None, sk=1, ts=1, pp=1, pc=None, allin=16, rr=1, wr=tuple(range(12)), nobc=True, big=False):
    def fn(x, g, b, w):
        B, S, D = x.shape
        H, Q = D // 2, D // 4
        G = B // NG
        NV = NG // 128
        RS0, XC0 = 64, 128
        TS = D + 9 * 8 * sk + 8 * ts
        ACC_HI = XC0 + 2 * NV * TS
        crow = lambda par, u, r: XC0 + (par * NV + u) * TS + r + (r // 64) * 8 * sk

        def kern(x_hbm, g_hbm, b_hbm, w_hbm, o_hbm, xbuf, obuf, wbuf, gbuf, bbuf, lhs, bias, cen, part, isem, osem, psem):
            starts = list(itertools.accumulate([0] + [n for n, reps in blocks for _ in range(reps)]))
            waited = [0] + [S - 1 if s0 >= allin else min(s1, S - 1) for s0, s1 in zip(starts[1:-1], starts[2:])]
            edges = sorted(set(waited))[1:-1]
            def stripes(src, dst, s, sem, part=0, parts=1):
                n = H // dr // parts
                for o in range(part * n * dr, (part + 1) * n * dr, dr):
                    for p in range(2):
                        sl = (s, pl.ds(p * H + o, dr))
                        pltpu.make_async_copy(src.at[sl], dst.at[sl], sem).start(priority=p)
            read_sem = lambda s: isem.at[G + add_all([0] + [(s > e).astype(jnp.int32) for e in edges])]
            def read_slab(s):
                stripes(x_hbm, xbuf, s, read_sem(s))
            def x_copy(k):
                sl = (0, slice(None), pl.ds(k * NG, NG))
                return pltpu.make_async_copy(x_hbm.at[sl], xbuf.at[sl], isem.at[k])
            params = [pltpu.make_async_copy(s, d, psem.at[0]) for s, d in ((g_hbm, gbuf), (b_hbm, bbuf), (w_hbm, wbuf))]
            for c in params:
                c.start()

            @pl.loop(0, G)
            def _(k):
                sl = (0, slice(None), pl.ds(pl.multiple_of(k * NG, NG), NG))
                pltpu.make_async_copy(x_hbm.at[sl], xbuf.at[sl], isem.at[k]).start()

            if dma:
                @pl.loop(1, lead)
                def _(s):
                    if big: pltpu.make_async_copy(x_hbm.at[s], xbuf.at[s], read_sem(s)).start()
                    else: read_slab(s)

            for c in params:
                c.wait()

            gr = gbuf[...].astype(F32).reshape(1, D)
            br = bbuf[...].astype(F32).reshape(1, D)
            lo = lax.broadcasted_iota(jnp.int32, (H, 128), 1) < 64
            A1, A2, c = [], [], None
            for t in range(5):
                if t < 4:
                    wt, gt, bt = wbuf[t * 128:(t + 1) * 128, :], gr[:, t * 128:(t + 1) * 128], br[:, t * 128:(t + 1) * 128]
                else:
                    wt = cat0([wbuf[512:, :]] * 2)
                    gt = cat1([gr[:, 512:]] * 2)
                    bt = cat1([br[:, 512:], jnp.zeros((1, 64), F32)])
                a = wt.astype(F32).T
                c = a * bt if c is None else c + a * bt
                a = a * gt
                A1.append(a[:H]); A2.append(a[H:])
            c = jnp.sum(c, axis=1, keepdims=True)
            bias[0] = jnp.broadcast_to(c[:H], (H, 128))
            bias[1] = jnp.broadcast_to(c[H:] - c[:H], (H, 128))
            sel = lambda u, v: jnp.where(lo, v, u)
            S1a, S1b = A2[0] + A2[1], A2[2] + A2[3]
            S2a, S2b = S1a - A1[0], S1b - A1[2]
            L = {"1a": A1[0], "1b": sel(A1[2], 0.0), "6a": S2a, "6b": sel(S2b, A2[4]),
                 "7a": A1[0] - A2[0], "7b": sel(A1[2] - A2[2], A2[3]), "5a": S1a, "5b": sel(S1b, A2[2]),
                 "2a": A1[1], "2b": A1[3], "2c": sel(A1[4], A1[2]),
                 "3c": A1[1] - S2a, "3b": sel(A1[3] - S2b, A1[3]), "3a": sel(A1[4] - A2[4], A1[2] - A2[2]),
                 "4c": A2[1], "4b": A2[3], "4a": sel(A2[4], A2[2])}
            for i, t in enumerate(FULL):
                lhs[i * Q:(i + 1) * Q] = pltpu.bitcast(L[t].astype(BF16), U32)
            sub0 = lambda p, i: len(FULL) * Q + ((int(p) - 1) * 7 + i - 1) * (Q // 2)
            for p in "1234":
                for i in L2:
                    v = None
                    for t, m, sg in L2[i][0]:
                        u = L[p + t][m * Q:(m + 1) * Q]
                        v = u if v is None else (v + u if sg > 0 else v - u)
                    lhs[sub0(p, i):sub0(p, i) + Q // 2] = pltpu.bitcast(v.astype(BF16), U32)

            def stats_work(s, gi, par, acc_base):
                acc_ref = cen.at[pl.ds(acc_base, 64)]
                wide = lambda v: cat1([v[8 * j:8 * j + 8] for j in range(NV)])
                tall = lambda v: cat0([v[:, 128 * j:128 * j + 128] for j in range(NV)])
                ld = lambda r0, n: xbuf[s, pl.ds(r0, n), pl.ds(gi * NG, NG)].astype(F32)
                def p1(r0):
                    v = ld(r0, r1)
                    v = add_all([v[i:i + 8] for i in range(0, r1, 8)])
                    acc = v if r0 == 0 else wide(acc_ref[0:32]) + v
                    if r0 + r1 == D:
                        acc = jnp.broadcast_to(jnp.sum(acc, axis=0, keepdims=True) * (1.0 / D), (8, NG))
                    acc_ref[0:32] = tall(acc)
                def p2(r0):
                    m = wide(acc_ref[0:32])
                    v = ld(r0, r2)
                    d = [v[i:i + 8] - m for i in range(0, r2, 8)]
                    for j in range(NV):
                        o = crow(par, j, r0)
                        cen[o:o + r2] = cat0([u[:, 128 * j:128 * j + 128] for u in d])
                    sq = add_all([u * u for u in d])
                    acc = sq if r0 == 0 else wide(acc_ref[32:64]) + sq
                    if r0 + r2 == D:
                        var = jnp.sum(acc, axis=0, keepdims=True) * (1.0 / D)
                        acc = jnp.broadcast_to(lax.rsqrt(var + EPS), (8, NG))
                        cen[RS0 + 32 * par:RS0 + 32 * par + 32] = tall(acc)
                    acc_ref[32:64] = tall(acc)
                P = functools.partial
                return [(2 * r1, P(p1, r0)) for r0 in range(0, D, r1)] + [(4 * r2, P(p2, r0)) for r0 in range(0, D, r2)]

            def rhs_tiles(par, tiles, hook):
                def signed_sum(terms):
                    terms = sorted(terms, key=lambda t: -t[0])
                    flip = terms[0][0]
                    v = terms[0][1]
                    for sg, u in terms[1:]:
                        v = v + u if sg == flip else v - u
                    return flip, v
                def piece(form, o):
                    if not form:
                        return jnp.zeros((jr, 128), F32)
                    terms = []
                    for u in sorted({k[0] for k in form}):
                        sg, v = signed_sum([(sg, cen[pl.ds(crow(par, u, r + o), jr)]) for (uu, r), sg in form.items() if uu == u])
                        rs = cen[RS0 + 32 * par + 8 * u:RS0 + 32 * par + 8 * u + 8]
                        terms.append((sg, v * cat0([rs] * (jr // 8))))
                    sg, v = signed_sum(terms)
                    assert sg > 0
                    return v
                n = 128 // jr
                v = [[None] * n for _ in tiles]
                for i in reversed(range(n)):
                    for j, t in enumerate(tiles):
                        if j == 0: hook()
                        v[j][i] = piece(t[i * jr // 64], i * jr % 64)
                return [cat0(u) for u in v]

            def group(s, gi, par, bank, side, fine, io):
                def out(r0, h, v):
                    sl = (s, pl.ds(r0, v.shape[0]), pl.ds(gi * NG + h * 256, 256))
                    obuf[sl] = v.astype(BF16)
                    if fine and dma:
                        @pl.when(s == S - 1)
                        def _(): pltpu.make_async_copy(obuf.at[sl], o_hbm.at[sl], osem.at[0]).start()
                if pc is None:
                    P1, U2, U3, Z2, Z3 = (part.at[bank, k, 0:H] for k in range(5))
                    quad = lambda ref, p, m, j: ref.at[m * Q:(m + 1) * Q, (j ^ SWAP[p]) * 128:((j ^ SWAP[p]) + 1) * 128]
                else:
                    class Part:
                        def __init__(self, k): self.c = [part.at[bank, pl.ds((2 * k + j) * (H + 32) + 8 * ((pc[0] * k + pc[1] * j) % 4), H)] for j in range(2)]
                        def __getitem__(self, _): return cat1([c[...] for c in self.c])
                        def __setitem__(self, _, v):
                            for j, c in enumerate(self.c): c[...] = v[:, j * 128:(j + 1) * 128]
                    P1, U2, U3, Z2, Z3 = (Part(k) for k in range(5))
                    quad = lambda ref, p, m, j: ref.c[j ^ SWAP[p]].at[m * Q:(m + 1) * Q]
                def four(p, n2, n3, n4, n5):
                    q = [[n4 - n5, n3 + n5], [n2 + n4, n3 - n2]]
                    return cat0([cat1(r[::-1] if SWAP[p] else r) for r in q])
                def diag(ref, p, a, b):
                    for m, v in enumerate((a, b)):
                        if v is not None:
                            r = quad(ref, p, m, m)
                            r[...] = r[...] + v
                two = lambda i: cat1([bias[i]] * 2)
                def r1_(a, b): Z2[...] = a; Z3[...] = b
                def a1(*n): P1[...] = two(0) + four("1", *n)
                def b1(n1, n7, n6, e): diag(P1, "1", n1 + n7, n1 + n6); diag(Z2, "2", e, None)
                def r6(a, b): U2[...] = P1[...] + (a + b)
                def r7(a, b): U3[...] = U2[...] + (a + b) + two(1)
                def r5(a, b):
                    m5 = a + b
                    out(H, 1, U3[...] + m5)
                    Z3[...] = Z3[...] + U2[...] + m5
                def b3(n1, n7, n6, e): diag(Z3, "3", n1 + n7, n1 + n6); diag(Z2, "2", None, e)
                def a3(*n): out(0, 1, Z3[...] + four("3", *n))
                def rc(a, b): U3[...] = U3[...] + cat0([a, b])
                def b4(n1, n7, n6, e): diag(U3, "4", n1 + n7, n1 + n6); diag(Z2, "2", e, e)
                def a2(*n): out(0, 0, (P1[...] + Z2[...]) + four("2", *n))
                def a4(*n): out(H, 0, U3[...] + four("4", *n))
                sa = lambda p: [(p, i) for i in (2, 3, 4, 5)]
                sb = lambda p, e: [(p, 1), (p, 7), (p, 6), ("2", e)]
                rounds = [(["2c", "3c"], r1_), (sa("1"), a1), (sb("1", 7), b1), (["6a", "6b"], r6), (["7a", "7b"], r7), (["5a", "5b"], r5),
                          (sb("3", 6), b3), (sa("3"), a3), (sb("4", 1), b4), (["4c"], rc), (sa("2"), a2), (sa("4"), a4)]
                total = sum(wt for wt, _ in side)
                cum = list(itertools.accumulate(rw[k] for k, (names, _) in enumerate(rounds) for _ in range(128 // jr)))
                st = dict(slot=0, pos=0, done=0)
                def hook():
                    want = cum[st["slot"]] * total / cum[-1] - 1e-6
                    st["slot"] += 1
                    while st["done"] < want:
                        wt, f = side[st["pos"]]
                        st["pos"] += 1; st["done"] += wt
                        f()
                mm = lambda o, n, v: jnp.dot(pltpu.bitcast(lhs[o:o + n // 2], BF16), v.astype(BF16), preferred_element_type=F32)
                for k, (names, post) in enumerate(rounds):
                    io(k)
                    if len(names) == 4:
                        v = rhs_tiles(par, [_rhs2(*t) for t in names], hook)
                        post(*(mm(sub0(*t), Q, u) for t, u in zip(names, v)))
                    else:
                        v = rhs_tiles(par, [_rhs(t, j) for t in names for j in range(2)], hook)
                        if len(names) == 2:
                            post(*(mm(FULL.index(t) * Q, H, cat1(v[2 * k:2 * k + 2])) for k, t in enumerate(names)))
                        else:
                            post(*(mm(FULL.index(names[0]) * Q + m * (Q // 2), Q, cat1(v)) for m in range(2)))
                assert st["pos"] == len(side)

            def block(it, s0, nslab, first, last):
                acc_base = pl.multiple_of(jnp.minimum(it * (ACC_HI // 8), ACC_HI // 8) * 8, 8)
                bank = it & 1
                for q in range(nslab * G):
                    ds, gi = divmod(q, G)
                    dn, gn = divmod(q + 1, G)
                    if dn < nslab: side = stats_work(s0 + dn, gn, (q + 1) % 2, acc_base)
                    else: side = stats_work(jnp.where(it == 0, 0, jnp.minimum(s0 + dn, S - 1)), gn, (q + 1) % 2, acc_base)
                    step = s0 * G + q
                    final = last == S and q == nslab * G - 1
                    if dma and rr and first * G + q + lead < S:
                        rs = jnp.minimum(step + lead, S - 1)
                        rsem = read_sem(rs)
                        nd = D // dr
                        def with_reads(f, ds_, rs=rs, rsem=rsem, step=step):
                            def g():
                                @pl.when(step + lead < S)
                                def _():
                                    for d in ds_:
                                        sl = (rs, pl.ds((d % 2) * H + (d // 2) * dr, dr))
                                        pltpu.make_async_copy(x_hbm.at[sl], xbuf.at[sl], rsem).start(priority=d % 2)
                                f()
                            return g
                        for i in range(len(side)):
                            ds_ = [d for d in range(nd) if (d // rr) * rr * len(side) // nd == i]
                            if ds_: side[i] = (side[i][0], with_reads(side[i][1], ds_))
                    def io(k):
                        if not dma: return
                        if k in wr and (last - nslab) * G + q >= wk:
                            done = s0 + ds - 1
                            cond = step >= wk
                            if gi > 0: cond = cond & (step - wk <= done)
                            @pl.when(cond)
                            def _(): stripes(obuf, o_hbm, jnp.clip(jnp.minimum(step - wk, done), 0, S - 1), osem.at[0], wr.index(k), len(wr))
                        if k == 0 and final:
                            @pl.when(s0 + ds == S - 1)
                            def _():
                                sl = (S - 1, slice(None), pl.ds(0, (G - 1) * NG))
                                pltpu.make_async_copy(obuf.at[sl], o_hbm.at[sl], osem.at[0]).start()
                    group(s0 + ds, gi, q % 2, bank, side, final, io)

            x_copy(0).wait()
            for _, f in stats_work(0, 0, 0, 0): f()
            for k in range(1, G): x_copy(k).wait()

            @pl.loop(0, len(starts) - 1)
            def _(it):
                for i in range(1, len(waited)):
                    if dma and waited[i] > waited[i - 1]:
                        @pl.when(it == i)
                        def _():
                            sl = pl.ds(waited[i - 1] + 1, waited[i] - waited[i - 1])
                            pltpu.make_async_copy(x_hbm.at[sl], xbuf.at[sl], isem.at[G + i - 1]).wait()
                @pl.when(it == 1)
                def _():
                    for _, f in stats_work(starts[1], 0, 0, 0): f()
                it0 = 0
                for nslab, reps in blocks:
                    @pl.when((it >= it0) & (it < it0 + reps))
                    def _():
                        block(it, starts[it0] + (it - it0) * nslab, nslab, starts[it0], starts[it0 + reps])
                    it0 += reps

            if dma:
                pltpu.make_async_copy(obuf, o_hbm, osem.at[0]).wait()
            else:
                c = pltpu.make_async_copy(obuf.at[0, pl.ds(0, 16)], o_hbm.at[0, pl.ds(0, 16)], osem.at[0]); c.start(); c.wait()

        st_ = list(itertools.accumulate([0] + [n for n, reps in blocks for _ in range(reps)]))
        assert st_[-1] == S and blocks[0][0] == 1
        nsem = len({S - 1 if s0 >= allin else min(s1, S - 1) for s0, s1 in zip(st_[1:-1], st_[2:])})
        for s0, s1 in zip(st_[1:-1], st_[2:]):
            assert (S - 1 if s0 >= allin else min(s1, S - 1)) - lead < G * s0, "read must be issued before its wait"
        hbm = pl.BlockSpec(memory_space=pl.ANY)
        out = pl.pallas_call(
            kern,
            in_specs=[hbm] * 4,
            out_specs=hbm,
            out_shape=jax.ShapeDtypeStruct((S, D, B), x.dtype),
            scratch_shapes=[pltpu.VMEM((S, D, B), BF16), pltpu.VMEM((S, D, B), BF16), pltpu.VMEM((D, D), BF16),
                            pltpu.VMEM((D,), BF16), pltpu.VMEM((D,), BF16),
                            pltpu.VMEM(((len(FULL) + 14) * Q, 128), U32), pltpu.VMEM((2, H, 128), F32), pltpu.VMEM((ACC_HI + 64, 128), F32),
                            pltpu.VMEM((2, 5, H + 8 * pp, 256) if pc is None else (2, 10 * (H + 32), 128), F32),
                            pltpu.SemaphoreType.DMA((G + nsem,)), pltpu.SemaphoreType.DMA((1,)), pltpu.SemaphoreType.DMA((1,))],
            compiler_params=pltpu.CompilerParams(vmem_limit_bytes=110 << 20, flags=flags, disable_bounds_checks=nobc),
        )(jnp.transpose(x, (1, 2, 0)), g, b, w)
        return jnp.transpose(out, (2, 0, 1))
    return fn


_impl = make(lead=32, big=True)


@jax.jit
def pallas_standalone__layernorm_linear__sampling_kernel(x, g, b, w):
    return _impl(x, g, b, w)
```

```python
import functools
import itertools

import jax
import jax.numpy as jnp
from jax import lax
import jax.experimental.pallas as pl
import jax.experimental.pallas.tpu as pltpu

F32, BF16, U32 = jnp.float32, jnp.bfloat16, jnp.uint32
EPS = 1e-5
LANES = 128
GROUP = 512
NTILE = GROUP // LANES

BLOCKS = ((1, 1), (1, 1), (2, 1), (4, 3), (16, 3))
WHOLE_SLABS = 5
READ_LEAD = 3
ALL_IN = 32
WRITE_STEP = 29
TAIL_SLABS = 2
STRIPE = 24
SUM_ROWS, VAR_ROWS = 64, 32
PIECE_SLOTS = (8, 8, 9, 13, 15, 15, 16, 18, 18, 20, 32, 33, 34, 36, 37, 39, 40, 41,
               42, 42, 43, 47, 48, 52, 54, 56, 60)

_FORMS = {
    "X1": lambda r: {(0, r): 1},
    "X2": lambda r: {(1, r): 1},
    "X2-X1": lambda r: {(1, r): 1, (0, r): -1},
    "X1-X2": lambda r: {(0, r): 1, (1, r): -1},
    "T2": lambda r: {(1, r + 128): 1, (1, r): -1, (0, r): 1},
    "T3": lambda r: {(1, r + 128): 1, (1, r): -1},
    "T4": lambda r: {(0, r + 128): 1, (0, r): -1, (1, r + 128): -1, (1, r): 1},
}
_LEVEL1 = {
    "1a": (("X1", 0), ("X1", 64)), "1b": (("0", 0), ("X1", 320)),
    "2a": (("X1", 128), ("X1", 192)), "2b": (("X1", 384), ("X1", 448)), "2c": (("X1", 256), ("X1", 512)),
    "3a": (("X2", 256), ("X2", 512)), "3b": (("X2", 384), ("X2", 448)), "3c": (("X2", 128), ("X2", 192)),
    "4a": (("X1", 256), ("X1-X2", 512)), "4b": (("X1-X2", 384), ("T4", 320)), "4c": (("T4", 0), ("T4", 64)),
    "5a": (("X2-X1", 0), ("X2-X1", 64)), "5b": (("X2", 256), ("X2-X1", 320)),
    "6a": (("T2", 0), ("T2", 64)), "6b": (("X2", 512), ("T2", 320)),
    "7a": (("T3", 0), ("T3", 64)), "7b": (("X2", 384), ("T3", 320)),
}
_FULL_TILES = ("2c", "3c", "4c", "5a", "5b", "6a", "6b", "7a", "7b")

_LEVEL2 = {
    1: ((("a", 0, 1), ("b", 1, 1)), (("a", 0, 1), ("b", 1, 1))),
    2: ((("a", 1, 1), ("b", 1, 1)), (("a", 0, 1),)),
    3: ((("a", 0, 1),), (("a", 1, 1), ("b", 1, -1))),
    4: ((("b", 1, 1),), (("b", 0, 1), ("a", 0, -1))),
    5: ((("a", 0, 1), ("b", 0, 1)), (("b", 1, 1),)),
    6: ((("a", 1, 1), ("a", 0, -1)), (("a", 0, 1), ("a", 1, 1))),
    7: ((("b", 0, 1), ("b", 1, -1)), (("b", 0, 1), ("b", 1, 1))),
}
_SWAP = {"1": 1, "2": 0, "3": 0, "4": 0}


def _level1_rhs(tile, j):
    return [[(1, (form, row, j))] for form, row in _LEVEL1[tile]]


def _level2_rhs(prod, i):
    lhs_terms, rhs_terms = _LEVEL2[i]
    return [[(sign, (*_LEVEL1[prod + t][k], j ^ _SWAP[prod])) for t, j, sign in rhs_terms
             if _LEVEL1[prod + t][k][0] != "0"]
            if any(_LEVEL1[prod + t][k][0] != "0" for t, _, _ in lhs_terms) else []
            for k in range(2)]


def _cat(xs, axis):
    return jnp.concatenate(xs, axis=axis) if len(xs) > 1 else xs[0]


def _total(xs):
    return functools.reduce(lambda a, b: a + b, xs)


def _signed_total(terms):
    (first, acc), *rest = sorted(terms, key=lambda t: -t[0])
    for sign, v in rest:
        acc = acc + v if sign == first else acc - v
    return first, acc


def _positive_total(terms):
    sign, v = _signed_total(terms)
    assert sign > 0
    return v


def _layernorm_linear(xt, g, b, w):
    S, D, B = xt.shape
    assert (D, B) == (576, 2 * GROUP)
    H, Q = D // 2, D // 4
    n_groups, n_copies = 2 * S, D // STRIPE

    starts = list(itertools.accumulate([0] + [n for n, reps in BLOCKS for _ in range(reps)]))
    arrived = [S - 1 if k0 >= ALL_IN else min(k1 // 2, S - 1) for k0, k1 in zip(starts, starts[1:])]
    edges = sorted(set(arrived))
    assert starts[-1] == n_groups and arrived[0] == 0
    assert all(s < max(k0 + READ_LEAD - 1, WHOLE_SLABS) for k0, s in zip(starts, arrived))
    assert READ_LEAD <= WHOLE_SLABS and 2 * TAIL_SLABS <= BLOCKS[-1][0]
    assert WRITE_STEP + S - TAIL_SLABS <= n_groups

    acc_lo = 16
    rstd_row = lambda slot, u: 96 + 32 * slot + 8 * u
    tile_rows = D + D // 8
    cen_row = lambda slot, u, r: 160 + acc_lo + (slot * NTILE + u) * tile_rows + r + r // 64 * 8
    acc_hi = cen_row(2, 0, 0)
    full_row = lambda tile: _FULL_TILES.index(tile) * Q
    sub_row = lambda prod, i: len(_FULL_TILES) * Q + ((int(prod) - 1) * 7 + i - 1) * (Q // 2)

    def kernel(x_hbm, g_hbm, b_hbm, w_hbm, o_hbm,
               xbuf, obuf, wbuf, gbuf, bbuf, lhs, bias, cen, part, xsem, osem, wsem):
        def copy_in(idx, sem):
            return pltpu.make_async_copy(x_hbm.at[idx], xbuf.at[idx], sem)

        def copy_out(idx):
            return pltpu.make_async_copy(obuf.at[idx], o_hbm.at[idx], osem.at[0])

        def slab_sem(s):
            return xsem.at[1 + _total([(s > e).astype(jnp.int32) for e in edges[:-1]])]

        def stripe(i):
            return pl.ds(i % 2 * H + i // 2 * STRIPE, STRIPE)

        def prepare_weights():
            g_row = gbuf[...].astype(F32).reshape(1, D)
            b_row = bbuf[...].astype(F32).reshape(1, D)
            a1, a2, c = [], [], []
            for k in range(0, D, LANES):
                if k + LANES <= D:
                    wk, gk, bk = wbuf[k:k + LANES, :], g_row[:, k:k + LANES], b_row[:, k:k + LANES]
                else:
                    wk = _cat([wbuf[k:, :]] * 2, 0)
                    gk = _cat([g_row[:, k:]] * 2, 1)
                    bk = _cat([b_row[:, k:], jnp.zeros((1, LANES // 2), F32)], 1)
                wt = wk.astype(F32).T
                c.append(wt * bk)
                a = wt * gk
                a1.append(a[:H])
                a2.append(a[H:])
            c = jnp.sum(_total(c), axis=1, keepdims=True)
            bias[0, 0:H] = jnp.broadcast_to(c[:H], (H, LANES))
            bias[1, 0:H] = jnp.broadcast_to(c[H:] - c[:H], (H, LANES))
            low = lax.broadcasted_iota(jnp.int32, (H, LANES), 1) < LANES // 2
            both = functools.partial(jnp.where, low)
            s1a, s1b = a2[0] + a2[1], a2[2] + a2[3]
            s2a, s2b = s1a - a1[0], s1b - a1[2]
            tiles = {
                "1a": a1[0], "1b": both(0.0, a1[2]),
                "2a": a1[1], "2b": a1[3], "2c": both(a1[2], a1[4]),
                "3a": both(a1[2] - a2[2], a1[4] - a2[4]), "3b": both(a1[3], a1[3] - s2b), "3c": a1[1] - s2a,
                "4a": both(a2[2], a2[4]), "4b": a2[3], "4c": a2[1],
                "5a": s1a, "5b": both(a2[2], s1b),
                "6a": s2a, "6b": both(a2[4], s2b),
                "7a": a1[0] - a2[0], "7b": both(a2[3], a1[2] - a2[2]),
            }
            for tile in _FULL_TILES:
                lhs[pl.ds(full_row(tile), Q)] = pltpu.bitcast(tiles[tile].astype(BF16), U32)
            for prod in _SWAP:
                for i, (terms, _) in _LEVEL2.items():
                    v = _positive_total([(sg, tiles[prod + t][m * Q:(m + 1) * Q]) for t, m, sg in terms])
                    lhs[pl.ds(sub_row(prod, i), Q // 2)] = pltpu.bitcast(v.astype(BF16), U32)

        def layernorm_pieces(s, slot, acc_row):
            acc = cen.at[pl.ds(acc_row, 64)]
            wide = lambda v: _cat([v[8 * u:8 * u + 8] for u in range(NTILE)], 1)
            tall = lambda v: _cat([v[:, u * LANES:(u + 1) * LANES] for u in range(NTILE)], 0)
            column_mean = lambda v: jnp.broadcast_to(jnp.sum(v, axis=0, keepdims=True) * (1.0 / D), v.shape)

            def load(r0, n):
                v = xbuf[s, pl.ds(r0, n), pl.ds(slot * GROUP, GROUP)].astype(F32)
                return v.reshape(n // 8, 8, GROUP)

            def add_rows(r0):
                v = jnp.sum(load(r0, SUM_ROWS), axis=0)
                if r0 > 0:
                    v = wide(acc[0:32]) + v
                acc[0:32] = tall(column_mean(v) if r0 + SUM_ROWS == D else v)

            def centre_rows(r0):
                mean = wide(acc[0:32])
                d = load(r0, VAR_ROWS) - mean
                rows = d.reshape(VAR_ROWS, GROUP)
                for u in range(NTILE):
                    cen[pl.ds(cen_row(slot, u, r0), VAR_ROWS)] = rows[:, u * LANES:(u + 1) * LANES]
                sq = jnp.sum(d * d, axis=0)
                if r0 > 0:
                    sq = wide(acc[32:64]) + sq
                if r0 + VAR_ROWS == D:
                    sq = lax.rsqrt(column_mean(sq) + EPS)
                    cen[pl.ds(rstd_row(slot, 0), 32)] = tall(sq)
                acc[32:64] = tall(sq)

            return ([functools.partial(add_rows, r) for r in range(0, D, SUM_ROWS)]
                    + [functools.partial(centre_rows, r) for r in range(0, D, VAR_ROWS)])

        def rhs_tiles(slot, tiles, side_work):
            def rows(r, n):
                @functools.cache
                def rstd(u):
                    return _cat([cen[pl.ds(rstd_row(slot, u), 8)]] * (n // 8), 0)

                @functools.cache
                def value(form, row, j):
                    form = _FORMS[form](row + r % 64)
                    terms = []
                    for half in sorted({h for h, _ in form}):
                        u = 2 * half + j
                        sign, v = _signed_total([(sg, cen[pl.ds(cen_row(slot, u, k), n)])
                                                 for (h, k), sg in form.items() if h == half])
                        terms.append((sign, v * rstd(u)))
                    return _positive_total(terms)

                return [_positive_total([(sign, value(*key)) for sign, key in tile[r // 64]])
                        if tile[r // 64] else jnp.zeros((n, LANES), F32) for tile in tiles]

            cuts = sorted({0, 4, 8, *side_work})
            out = []
            for i, j in zip(cuts, cuts[1:]):
                for work in side_work.get(i, ()):
                    work()
                out.insert(0, rows(LANES - 16 * j, 16 * (j - i)))
            return [_cat(col, 0) for col in zip(*out)]

        def multiply_group(s, slot, bank, pieces, before_round, quadrant_done):
            p1, u2, u3, z2, z3 = (part.at[bank, k, pl.ds(k % 2 * 8, H)] for k in range(5))
            wide_bias = lambda i: _cat([bias[i, 0:H]] * 2, 1)

            def emit(i, j, v):
                idx = (s, pl.ds(i * H, H), pl.ds(slot * GROUP + j * 2 * LANES, 2 * LANES))
                obuf[idx] = v.astype(obuf.dtype)
                quadrant_done(idx, j)

            def spread(prod, n2, n3, n4, n5):
                rows = [[n4 - n5, n3 + n5], [n2 + n4, n3 - n2]]
                return _cat([_cat(r[::-1] if _SWAP[prod] else r, 1) for r in rows], 0)

            def add_diagonal(ref, prod, *parts):
                for m, v in enumerate(parts):
                    if v is not None:
                        idx = (pl.ds(m * Q, Q), pl.ds((m ^ _SWAP[prod]) * LANES, LANES))
                        ref[idx] = ref[idx] + v

            def m23_c(a, b):
                z2[...] = a
                z3[...] = b

            def m1_spread(*n):
                p1[...] = wide_bias(0) + spread("1", *n)

            def m1_diagonal(n1, n7, n6, m2_n7):
                add_diagonal(p1, "1", n1 + n7, n1 + n6)
                add_diagonal(z2, "2", m2_n7, None)

            def m6(a, b):
                u2[...] = p1[...] + (a + b)

            def m7(a, b):
                u3[...] = u2[...] + (a + b) + wide_bias(1)

            def m5(a, b):
                v = a + b
                emit(1, 1, u3[...] + v)
                z3[...] = z3[...] + u2[...] + v

            def m3_diagonal(n1, n7, n6, m2_n6):
                add_diagonal(z3, "3", n1 + n7, n1 + n6)
                add_diagonal(z2, "2", None, m2_n6)

            def m3_spread(*n):
                emit(0, 1, z3[...] + spread("3", *n))

            def m4_diagonal(n1, n7, n6, m2_n1):
                add_diagonal(u3, "4", n1 + n7, n1 + n6)
                add_diagonal(z2, "2", m2_n1, m2_n1)

            def m2_spread(*n):
                emit(0, 0, (p1[...] + z2[...]) + spread("2", *n))

            def m4_spread(*n):
                u3[...] = u3[...] + spread("4", *n)

            def m4_c(top, bottom):
                emit(1, 0, u3[...] + _cat([top, bottom], 0))

            spreads = lambda prod: [(prod, i) for i in (2, 3, 4, 5)]
            diagonals = lambda prod, extra: [(prod, 1), (prod, 7), (prod, 6), ("2", extra)]
            rounds = [
                (["2c", "3c"], m23_c), (spreads("1"), m1_spread), (diagonals("1", 7), m1_diagonal),
                (["6a", "6b"], m6), (["7a", "7b"], m7), (["5a", "5b"], m5),
                (diagonals("3", 6), m3_diagonal), (spreads("3"), m3_spread), (diagonals("4", 1), m4_diagonal),
                (spreads("2"), m2_spread), (spreads("4"), m4_spread), (["4c"], m4_c),
            ]

            side_work = [{} for _ in rounds]
            for at, piece in zip(PIECE_SLOTS, pieces, strict=True):
                side_work[at // 8].setdefault(at % 8, []).append(piece)

            def matmul(row, n, v):
                a = pltpu.bitcast(lhs[pl.ds(row, n // 2)], BF16)
                return jnp.dot(a, v.astype(BF16), preferred_element_type=F32)

            for k, (tiles, combine) in enumerate(rounds):
                before_round(k, len(rounds))
                if len(tiles) == 4:
                    v = rhs_tiles(slot, [_level2_rhs(*t) for t in tiles], side_work[k])
                    combine(*(matmul(sub_row(*t), Q, u) for t, u in zip(tiles, v)))
                else:
                    v = rhs_tiles(slot, [_level1_rhs(t, j) for t in tiles for j in range(2)], side_work[k])
                    if len(tiles) == 2:
                        combine(*(matmul(full_row(t), H, _cat(v[2 * i:2 * i + 2], 1)) for i, t in enumerate(tiles)))
                    else:
                        combine(*(matmul(full_row(tiles[0]) + m * Q // 2, Q, _cat(v, 1)) for m in range(2)))

        def step(it, k0, q, n, first, last):
            slot = (first + q) % 2
            k = k0 + q
            s = k0 // 2 + (first % 2 + q) // 2
            s_next = s + slot if q + 1 < n or last + n < n_groups else jnp.minimum(s + slot, S - 1)
            acc_row = acc_lo + 8 * jnp.minimum(it * ((acc_hi - acc_lo) // 8), (acc_hi - acc_lo) // 8)
            pieces = layernorm_pieces(s_next, 1 - slot, pl.multiple_of(acc_row, 8))

            reading = max(first + READ_LEAD - 1, WHOLE_SLABS) < S and last + n + READ_LEAD > WHOLE_SLABS
            if reading:
                slabs = [k + READ_LEAD - 1, k + READ_LEAD]
                safe = [lax.rem(t, S) for t in slabs]
                sems = [slab_sem(t) for t in safe]
                go = [(t >= WHOLE_SLABS) & (t < S) for t in slabs]

                def read_then(i, piece):
                    new, i = divmod(i + n_copies // 2, n_copies)

                    @pl.when(go[new])
                    def _():
                        copy_in((safe[new], stripe(i)), sems[new]).start(priority=i % 2)
                    piece()

                for i in range(n_copies):
                    j = i * len(pieces) // n_copies
                    pieces[j] = functools.partial(read_then, i, pieces[j])

            writing = last + q >= WRITE_STEP
            if writing:
                done = jnp.minimum(k - WRITE_STEP, s - 1)
                write = (k >= WRITE_STEP) & (done < S - TAIL_SLABS)
                if slot:
                    write = write & (k - WRITE_STEP < s)
                done = jnp.clip(done, 0, S - 1)

            def before_round(r, n_rounds):
                if writing:
                    per_round = n_copies // n_rounds

                    @pl.when(write)
                    def _():
                        for i in range(r * per_round, (r + 1) * per_round):
                            copy_out((done, stripe(i))).start(priority=i % 2)

            def quadrant_done(idx, queue):
                if last + n == n_groups and q >= n - 2 * TAIL_SLABS:
                    @pl.when(k0 == last)
                    def _():
                        copy_out(idx).start(priority=queue)

            multiply_group(s, slot, it & 1, pieces, before_round, quadrant_done)

        first_group = lambda i: (0, slice(None), pl.ds(pl.multiple_of(i * GROUP, GROUP), GROUP))
        params = [pltpu.make_async_copy(src, dst, wsem.at[0])
                  for src, dst in ((g_hbm, gbuf), (b_hbm, bbuf), (w_hbm, wbuf))]
        for copy in params:
            copy.start()

        @pl.loop(0, 2)
        def _(i):
            copy_in(first_group(i), xsem.at[i]).start()

        @pl.loop(1, WHOLE_SLABS)
        def _(s):
            copy_in((s,), slab_sem(s)).start()

        for copy in params:
            copy.wait()
        prepare_weights()
        copy_in((0, slice(None), pl.ds(0, GROUP)), xsem.at[0]).wait()
        for piece in layernorm_pieces(0, 0, acc_lo):
            piece()
        copy_in((0, slice(None), pl.ds(GROUP, GROUP)), xsem.at[1]).wait()

        @pl.loop(0, len(arrived))
        def _(it):
            i0 = 0
            for n, reps in BLOCKS:
                assert reps == 1 or n % 2 == 0

                @pl.when((it >= i0) & (it < i0 + reps))
                def _():
                    for i in range(max(i0, 1), i0 + reps):
                        if arrived[i] > arrived[i - 1]:
                            slabs = pl.ds(arrived[i - 1] + 1, arrived[i] - arrived[i - 1])
                            copies = copy_in((slabs,), xsem.at[1 + edges.index(arrived[i])])
                            if reps == 1:
                                copies.wait()
                            else:
                                pl.when(it == i)(copies.wait)
                    k0 = starts[i0] + (it - i0) * n
                    for q in range(n):
                        step(it, k0, q, n, starts[i0], starts[i0 + reps - 1])
                i0 += reps

        pltpu.make_async_copy(obuf, o_hbm, osem.at[0]).wait()

    hbm = pl.BlockSpec(memory_space=pl.ANY)
    return pl.pallas_call(
        kernel,
        in_specs=[hbm] * 4,
        out_specs=hbm,
        out_shape=jax.ShapeDtypeStruct(xt.shape, xt.dtype),
        scratch_shapes=[
            pltpu.VMEM(xt.shape, xt.dtype),
            pltpu.VMEM(xt.shape, xt.dtype),
            pltpu.VMEM(w.shape, w.dtype),
            pltpu.VMEM(g.shape, g.dtype),
            pltpu.VMEM(b.shape, b.dtype),
            pltpu.VMEM((sub_row("5", 1) + 16, LANES), U32),
            pltpu.VMEM((2, H + 32, LANES), F32),
            pltpu.VMEM((acc_hi + 64, LANES), F32),
            pltpu.VMEM((2, 5, H + 16, 2 * LANES), F32),
            pltpu.SemaphoreType.DMA((len(edges) + 1,)),
            pltpu.SemaphoreType.DMA((1,)),
            pltpu.SemaphoreType.DMA((1,)),
        ],
        compiler_params=pltpu.CompilerParams(vmem_limit_bytes=100 << 20, disable_bounds_checks=True),
    )(xt, g, b, w)


@jax.jit
def pallas_standalone__layernorm_linear__sampling_kernel(
    x: jax.Array,
    g: jax.Array,
    b: jax.Array,
    w: jax.Array,
):
    out = _layernorm_linear(jnp.transpose(x, (1, 2, 0)), g, b, w)
    return jnp.transpose(out, (2, 0, 1))
```
